```python
import os as _os
_os.environ.setdefault("JAX_PLATFORMS", "cpu")
import jax
import jax.numpy as jnp

def _softmax(x, axis=-1):
    return jax.nn.softmax(x, axis=axis)
def _gelu(x):
    return jax.nn.gelu(x, approximate=True)
def _silu(x):
    return jax.nn.silu(x)
def _sigmoid(x):
    return jax.nn.sigmoid(x)
def _layernorm(x, axis=-1, eps=1e-5):
    m = jnp.mean(x, axis=axis, keepdims=True)
    v = jnp.var(x, axis=axis, keepdims=True)
    return (x - m) / jnp.sqrt(v + eps)
def _scatter_add(tgt, idx, src, axis=0):
    return tgt.at[idx].add(src)
def _segment_sum(src, seg, n):
    return jax.ops.segment_sum(src, seg, n)
class _Rng:
    def __init__(self, key):
        self._k = key
    def _next(self):
        self._k, sub = jax.random.split(self._k)
        return sub
    def normal(self, shape):
        return jax.random.normal(self._next(), shape, dtype=jnp.bfloat16)
    def randint(self, lo, hi, shape):
        return jax.random.randint(self._next(), shape, lo, hi, dtype=jnp.int32)
    def uniform(self, shape, lo=0.0, hi=1.0):
        return jax.random.uniform(self._next(), shape, jnp.bfloat16, lo, hi)
    def permutation(self, n):
        return jax.random.permutation(self._next(), n)


kernel_name = 'interleave_layers__gqa_block_cached__dense_activation_mish__decode'

def setup_inputs():
    _rng = _Rng(jax.random.key(int.from_bytes(__import__("os").urandom(4), "little")))
    _w = (lambda a: (lambda t: t.astype(jnp.bfloat16) if jnp.issubdtype(t.dtype, jnp.floating) else t)(jnp.asarray(a)))
    def _A_setup():
        B, Sq, D = 1, 1, 512
        Hq, Hkv, Sk, Dh = 32, 8, 65536, 128
        assert Hq % Hkv == 0, (Hq, Hkv)
        return {
            "x": _w((lambda *s: _rng.normal(s) * 0.05)(B, Sq, D)),
            "k_cache": _w((lambda *s: _rng.normal(s) * 1.6)(B, Hkv, Sk, Dh)),
            "v_cache": _w((lambda *s: _rng.normal(s) * 1.6)(B, Hkv, Sk, Dh)),
            "wq": _w((lambda *s: _rng.normal(s) * 1.6)(D, Hq * Dh) * (D ** -0.5)),
            "wo": _w((lambda *s: _rng.normal(s) * 1.6)(Hq * Dh, D) * ((Hq * Dh) ** -0.5)),
        }
    _A_in = _A_setup()

    def _B_setup():
        B, S, D, F = 1, 1, 512, 1792
        return {
            "x": _w((lambda *s: _rng.normal(s) * 0.05)(B, S, D)),
            "w1": _w((lambda *s: _rng.normal(s) * 0.8)(D, F) * (D ** -0.5)),
            "b1": _w((lambda *s: _rng.normal(s) * 0.8)(F)),
            "w2": _w((lambda *s: _rng.normal(s) * 0.8)(F, D) * (F ** -0.5)),
        }
    _B_in = _B_setup()

    return {
        "A_x": _A_in["x"],
        "A_k_cache": _A_in["k_cache"],
        "A_v_cache": _A_in["v_cache"],
        "A_wq": _A_in["wq"],
        "A_wo": _A_in["wo"],
        "B_x": _B_in["x"],
        "B_w1": _B_in["w1"],
        "B_b1": _B_in["b1"],
        "B_w2": _B_in["w2"],
    }

def reference(A_x, A_k_cache, A_v_cache, A_wq, A_wo, B_x, B_w1, B_b1, B_w2):
    def _A_ref(x, k_cache, v_cache, wq, wo):
        B, Sq, D = x.shape
        Hq, Dh = 32, 128
        Hkv = k_cache.shape[1]
        rep = Hq // Hkv
        q = (lambda x, *d: x.transpose(*d))((x @ wq).reshape(B, Sq, Hq, Dh), 0, 2, 1, 3)
        k = jnp.repeat(k_cache, rep, axis=1)
        v = jnp.repeat(v_cache, rep, axis=1)
        scores = jnp.einsum("bhqd,bhkd->bhqk", q, k) * (Dh ** -0.5)
        p = _softmax(scores, axis=-1)
        o = jnp.einsum("bhqk,bhkd->bhqd", p, v)
        return (lambda x, *d: x.transpose(*d))(o, 0, 2, 1, 3).reshape(B, Sq, Hq * Dh) @ wo

    def _B_ref(x, w1, b1, w2):
        h = jnp.einsum("bsd,df->bsf", x, w1) + b1
        sp = jnp.log1p(jnp.exp(-jnp.abs(h))) + jnp.where(h > 0, h, jnp.zeros_like(h))
        act = h * jnp.tanh(sp)
        return jnp.einsum("bsf,fd->bsd", act, w2)

    x = A_x
    x = x + _A_ref(_layernorm(x, axis=-1), A_k_cache, A_v_cache, A_wq, A_wo)
    x = x + _B_ref(_layernorm(x, axis=-1), B_w1, B_b1, B_w2)
    x = x + _A_ref(_layernorm(x, axis=-1), A_k_cache, A_v_cache, A_wq, A_wo)
    x = x + _B_ref(_layernorm(x, axis=-1), B_w1, B_b1, B_w2)
    return x
```

```python
import functools

import numpy as np
import jax
import jax.numpy as jnp
from jax import lax
import jax.experimental.pallas as pl
import jax.experimental.pallas.tpu as pltpu

HQ = 32
DH = 128
EPS = 1e-5

TK = 2048
NR = 3
NC = 112
VMEM_LIMIT = 128 * 1024 * 1024


def _make_tables(nblk, nc, nr):
    ns = nblk - nc
    if ns > 1:
        spos = [(s * (nblk - 1)) // (ns - 1) for s in range(ns)]
    else:
        spos = [nblk - 1] * ns
    assert len(set(spos)) == ns
    streamed = np.zeros(nblk, bool)
    streamed[spos] = True
    slot1 = np.zeros(nblk, np.int32)
    slot2 = np.zeros(nblk, np.int32)
    g2 = np.full(nblk, -1, np.int32)
    ng = nblk + ns
    dma_blk = np.zeros(ng, np.int32)
    dma_slot = np.zeros(ng, np.int32)
    ci = 0
    si = 0
    for t in range(nblk):
        if streamed[t]:
            slot1[t] = nc + si % nr
            si += 1
        else:
            slot1[t] = ci
            slot2[t] = ci
            ci += 1
        dma_blk[t] = t
        dma_slot[t] = slot1[t]
    for j, t in enumerate(spos):
        s = ns + j
        slot2[t] = nc + s % nr
        g2[t] = nblk + j
        dma_blk[nblk + j] = t
        dma_slot[nblk + j] = slot2[t]
    return slot1, slot2, g2, dma_blk, dma_slot, ng


def _layernorm_bf16(x):
    m = jnp.mean(x, axis=-1, keepdims=True)
    d = x - m
    v = jnp.mean(d * d, axis=-1, keepdims=True)
    return (d / jnp.sqrt(v + EPS)).astype(jnp.bfloat16)


def _rb(x):
    return x.astype(jnp.bfloat16).astype(jnp.float32)


def _kernel(slot1_ref, slot2_ref, g2_ref, dblk_ref, dslot_ref,
            x_hbm, k_hbm, v_hbm, wq_hbm, wo_hbm, w1_hbm, b1_hbm, w2_hbm,
            o_ref,
            kpool, vpool, x_v, wq_v, wo_v, w1_v, b1_v, w2_v, q_scr,
            semk, semv, semw,
            *, hkv, nch, ng, d_model):
    rep = HQ // hkv
    nblk = hkv * nch
    scale = DH ** -0.5

    def kv_copies(g):
        blk = dblk_ref[g]
        slot = dslot_ref[g]
        si = lax.rem(g, NR)
        off = pl.multiple_of(blk * TK, TK)
        ck = pltpu.make_async_copy(k_hbm.at[pl.ds(off, TK)], kpool.at[slot], semk.at[si])
        cv = pltpu.make_async_copy(v_hbm.at[pl.ds(off, TK)], vpool.at[slot], semv.at[si])
        return ck, cv

    def issue(g):
        ck, cv = kv_copies(g)
        ck.start()
        cv.start()

    w_copies = [
        pltpu.make_async_copy(x_hbm, x_v, semw.at[0]),
        pltpu.make_async_copy(wq_hbm, wq_v, semw.at[1]),
        pltpu.make_async_copy(wo_hbm, wo_v, semw.at[2]),
        pltpu.make_async_copy(w1_hbm, w1_v, semw.at[3]),
        pltpu.make_async_copy(b1_hbm, b1_v, semw.at[4]),
        pltpu.make_async_copy(w2_hbm, w2_v, semw.at[5]),
    ]
    w_copies[0].start()
    w_copies[1].start()
    for g in range(NR):
        issue(g)
    for c in w_copies[2:]:
        c.start()

    row = lax.broadcasted_iota(jnp.int32, (8, DH), 0)

    def compute_q(x):
        xn = _layernorm_bf16(x)
        qf = jnp.dot(xn, wq_v[...], preferred_element_type=jnp.float32)
        for h in range(hkv):
            qh = jnp.zeros((8, DH), jnp.float32)
            for r in range(rep):
                j = h * rep + r
                qh = jnp.where(row == r, qf[:, j * DH:(j + 1) * DH], qh)
            q_scr[h] = qh.astype(jnp.bfloat16)

    def attention(layer):
        slot_ref = slot1_ref if layer == 0 else slot2_ref

        def head_body(h, att):
            q = q_scr[h]

            def chunk_body(c, carry):
                m, l, acc = carry
                t = h * nch + c
                slot = slot_ref[t]
                if layer == 0:
                    g = t
                    ck, cv = kv_copies(g)
                    ck.wait()
                else:
                    g = g2_ref[t]

                    @pl.when(g >= 0)
                    def _():
                        ck, _cv = kv_copies(g)
                        ck.wait()

                k = kpool[slot]
                s = lax.dot_general(q, k, (((1,), (1,)), ((), ())),
                                    preferred_element_type=jnp.float32)
                s = s * scale
                m_new = jnp.maximum(m, jnp.max(s, axis=-1, keepdims=True))
                alpha = jnp.exp(m - m_new)
                p = jnp.exp(s - m_new)
                ps = p[:, 0:DH]
                for i in range(1, TK // DH):
                    ps = ps + p[:, i * DH:(i + 1) * DH]
                l = l * alpha + ps

                if layer == 0:
                    cv.wait()
                else:
                    @pl.when(g >= 0)
                    def _():
                        _ck, cv2 = kv_copies(g)
                        cv2.wait()

                v = vpool[slot]
                acc = acc * alpha + jnp.dot(p.astype(jnp.bfloat16), v,
                                            preferred_element_type=jnp.float32)

                if layer == 0:
                    issue(g + NR)
                else:
                    @pl.when(jnp.logical_and(g >= 0, g + NR < ng))
                    def _():
                        issue(g + NR)
                return m_new, l, acc

            m0 = jnp.full((8, 1), -jnp.inf, jnp.float32)
            l0 = jnp.zeros((8, DH), jnp.float32)
            a0 = jnp.zeros((8, DH), jnp.float32)
            m, l, acc = lax.fori_loop(0, nch, chunk_body, (m0, l0, a0))
            o = acc / jnp.sum(l, axis=-1, keepdims=True)
            lhs = jnp.concatenate(
                [jnp.where(row == r, o, 0.0) for r in range(rep)], axis=1
            ).astype(jnp.bfloat16)
            if layer == 0:
                @pl.when(h == 0)
                def _():
                    w_copies[2].wait()
            woh = wo_v[pl.ds(pl.multiple_of(h * (rep * DH), rep * DH), rep * DH), :]
            return att + jnp.dot(lhs, woh, preferred_element_type=jnp.float32)

        att = lax.fori_loop(0, hkv, head_body, jnp.zeros((8, d_model), jnp.float32))
        att = jnp.sum(att, axis=0, keepdims=True)
        return jnp.broadcast_to(att, (8, d_model))

    def mlp(x):
        xn = _layernorm_bf16(x)
        h = jnp.dot(xn, w1_v[...], preferred_element_type=jnp.float32)
        h = _rb(_rb(h) + b1_v[...].astype(jnp.float32))
        sp = jnp.log1p(jnp.exp(-jnp.abs(h))) + jnp.where(h > 0, h, 0.0)
        act = h * jnp.tanh(sp)
        return jnp.dot(act.astype(jnp.bfloat16), w2_v[...],
                       preferred_element_type=jnp.float32)

    w_copies[0].wait()
    w_copies[1].wait()
    x = jnp.broadcast_to(x_v[...].astype(jnp.float32), (8, d_model))

    compute_q(x)
    x = _rb(x + _rb(attention(0)))
    for c in w_copies[3:]:
        c.wait()
    x = _rb(x + _rb(mlp(x)))
    compute_q(x)
    x = _rb(x + _rb(attention(1)))
    x = _rb(x + _rb(mlp(x)))
    o_ref[...] = x[0:1, :].astype(o_ref.dtype)


@jax.jit
def pallas_interleave_layers__gqa_block_cached__dense_activation_mish__decode_kernel(
    A_x: jax.Array,
    A_k_cache: jax.Array,
    A_v_cache: jax.Array,
    A_wq: jax.Array,
    A_wo: jax.Array,
    B_x: jax.Array,
    B_w1: jax.Array,
    B_b1: jax.Array,
    B_w2: jax.Array,
):
    B, Sq, D = A_x.shape
    _, hkv, sk, dh = A_k_cache.shape
    assert B == 1 and Sq == 1 and dh == DH and sk % TK == 0
    F = B_w1.shape[1]
    nch = sk // TK
    nblk = hkv * nch
    slot1, slot2, g2, dblk, dslot, ng = _make_tables(nblk, NC, NR)

    x2 = A_x.reshape(1, D)
    k2 = A_k_cache.reshape(hkv * sk, DH)
    v2 = A_v_cache.reshape(hkv * sk, DH)
    b1 = B_b1.reshape(1, F)

    smem = pl.BlockSpec(memory_space=pltpu.SMEM)
    hbm = pl.BlockSpec(memory_space=pl.ANY)
    kernel = functools.partial(_kernel, hkv=hkv, nch=nch, ng=ng, d_model=D)
    out = pl.pallas_call(
        kernel,
        out_shape=jax.ShapeDtypeStruct((1, D), A_x.dtype),
        in_specs=[smem] * 5 + [hbm] * 8,
        out_specs=pl.BlockSpec(memory_space=pltpu.VMEM),
        scratch_shapes=[
            pltpu.VMEM((NC + NR, TK, DH), jnp.bfloat16),
            pltpu.VMEM((NC + NR, TK, DH), jnp.bfloat16),
            pltpu.VMEM((1, D), jnp.bfloat16),
            pltpu.VMEM(A_wq.shape, jnp.bfloat16),
            pltpu.VMEM(A_wo.shape, jnp.bfloat16),
            pltpu.VMEM(B_w1.shape, jnp.bfloat16),
            pltpu.VMEM((1, F), jnp.bfloat16),
            pltpu.VMEM(B_w2.shape, jnp.bfloat16),
            pltpu.VMEM((hkv, 8, DH), jnp.bfloat16),
            pltpu.SemaphoreType.DMA((NR,)),
            pltpu.SemaphoreType.DMA((NR,)),
            pltpu.SemaphoreType.DMA((6,)),
        ],
        compiler_params=pltpu.CompilerParams(vmem_limit_bytes=VMEM_LIMIT),
    )(jnp.asarray(slot1), jnp.asarray(slot2), jnp.asarray(g2), jnp.asarray(dblk),
      jnp.asarray(dslot), x2, k2, v2, A_wq, A_wo, B_w1, b1, B_w2)
    return out.reshape(B, Sq, D)
```

```python
import functools

import numpy as np
import jax
import jax.numpy as jnp
from jax import lax
import jax.experimental.pallas as pl
import jax.experimental.pallas.tpu as pltpu

HQ = 32
DH = 128
EPS = 1e-5

TK = 2048
NRU = 3
NCU = 229
VMEM_LIMIT = 128 * 1024 * 1024


def _stream_count(u, nu, ns):
    return (u * (ns - 1) + (nu - 2)) // (nu - 1)


def _make_tables(nu, nc, nr):
    ns = nu - nc
    spos = [(s * (nu - 1)) // (ns - 1) for s in range(ns)]
    assert len(set(spos)) == ns
    streamed = np.zeros(nu, bool)
    streamed[spos] = True
    for u in range(nu + 1):
        assert _stream_count(u, nu, ns) == int(streamed[:u].sum())
    ng = nu + ns
    dma_unit = np.zeros(ng, np.int32)
    dma_slot = np.zeros(ng, np.int32)
    ci = 0
    si = 0
    for u in range(nu):
        if streamed[u]:
            slot = nc + si % nr
            si += 1
        else:
            slot = ci
            ci += 1
        dma_unit[u] = u
        dma_slot[u] = slot
    for j, u in enumerate(spos):
        dma_unit[nu + j] = u
        dma_slot[nu + j] = nc + (ns + j) % nr
    return dma_unit, dma_slot


def _layernorm_bf16(x):
    m = jnp.mean(x, axis=-1, keepdims=True)
    d = x - m
    v = jnp.mean(d * d, axis=-1, keepdims=True)
    return (d / jnp.sqrt(v + EPS)).astype(jnp.bfloat16)


def _rb(x):
    return x.astype(jnp.bfloat16).astype(jnp.float32)


def _kernel(x_hbm, k_hbm, v_hbm, wq_hbm, wo_hbm, w1_hbm, b1_hbm, w2_hbm,
            o_ref,
            pool, x_v, wq_v, wo_v, w1_v, b1_v, w2_v,
            slot1_ref, slot2_ref, g2_ref, dunit_ref, dslot_ref,
            sem, semw,
            *, hkv, nch, d_model):
    rep = HQ // hkv
    nu = 2 * hkv * nch
    ns = nu - NCU
    ng = nu + ns
    scale = DH ** -0.5
    tabs = _make_tables(nu, NCU, NRU)
    srcs = (k_hbm, v_hbm)

    def unit_copy(g, which):
        if isinstance(g, int):
            blk = int(tabs[0][g]) // 2
            slot = int(tabs[1][g])
            si = g % NRU
            off = blk * TK
        else:
            blk = lax.shift_right_logical(dunit_ref[g], 1)
            slot = dslot_ref[g]
            si = lax.rem(g, NRU)
            off = pl.multiple_of(blk * TK, TK)
        return pltpu.make_async_copy(srcs[which].at[pl.ds(off, TK)], pool.at[slot],
                                     sem.at[si])

    def issue(g):
        if isinstance(g, int):
            unit_copy(g, int(tabs[0][g]) % 2).start()
            return
        par = jnp.bitwise_and(dunit_ref[g], 1)

        @pl.when(par == 0)
        def _():
            unit_copy(g, 0).start()

        @pl.when(par == 1)
        def _():
            unit_copy(g, 1).start()

    w_copies = [
        pltpu.make_async_copy(x_hbm, x_v, semw.at[0]),
        pltpu.make_async_copy(wq_hbm, wq_v, semw.at[1]),
        pltpu.make_async_copy(wo_hbm, wo_v, semw.at[2]),
        pltpu.make_async_copy(w1_hbm, w1_v, semw.at[3]),
        pltpu.make_async_copy(b1_hbm, b1_v, semw.at[4]),
        pltpu.make_async_copy(w2_hbm, w2_v, semw.at[5]),
    ]
    w_copies[0].start()
    w_copies[1].start()
    for g in range(NRU):
        issue(g)
    for c in w_copies[2:]:
        c.start()

    def fill(u, carry):
        c0 = _stream_count(u, nu, ns)
        c1 = _stream_count(u + 1, nu, ns)
        is_s = c1 > c0
        s1 = jnp.where(is_s, NCU + lax.rem(c0, NRU), u - c0)
        s2 = jnp.where(is_s, NCU + lax.rem(ns + c0, NRU), u - c0)
        slot1_ref[u] = s1
        slot2_ref[u] = s2
        g2_ref[u] = jnp.where(is_s, nu + c0, -1)
        dunit_ref[u] = u
        dslot_ref[u] = s1

        @pl.when(is_s)
        def _():
            dunit_ref[nu + c0] = u
            dslot_ref[nu + c0] = s2
        return carry

    lax.fori_loop(0, nu, fill, 0)

    row = lax.broadcasted_iota(jnp.int32, (8, DH), 0)

    def attention(layer, x):
        slot_ref = slot1_ref if layer == 0 else slot2_ref
        xn = _layernorm_bf16(x)

        def acquire(u, which):
            if layer == 0:
                unit_copy(u, which).wait()
                return u
            g = g2_ref[u]

            @pl.when(g >= 0)
            def _():
                unit_copy(g, which).wait()
            return g

        def release(g):
            if layer == 0:
                issue(g + NRU)
            else:
                @pl.when(jnp.logical_and(g >= 0, g + NRU < ng))
                def _():
                    issue(g + NRU)

        def head_body(h, att):
            col = pl.multiple_of(h * (rep * DH), rep * DH)
            qf = jnp.dot(xn, wq_v[:, pl.ds(col, rep * DH)],
                         preferred_element_type=jnp.float32)
            q = jnp.zeros((8, DH), jnp.float32)
            for r in range(rep):
                q = jnp.where(row == r, qf[:, r * DH:(r + 1) * DH], q)
            q = q.astype(jnp.bfloat16)

            def chunk_body(c, carry):
                m, l, acc = carry
                u = 2 * (h * nch + c)
                g = acquire(u, 0)
                k = pool[slot_ref[u]]
                s = lax.dot_general(q, k, (((1,), (1,)), ((), ())),
                                    preferred_element_type=jnp.float32)
                release(g)
                s = s * scale
                m_new = jnp.maximum(m, jnp.max(s, axis=-1, keepdims=True))
                alpha = jnp.exp(m - m_new)
                p = jnp.exp(s - m_new)
                ps = p[:, 0:DH]
                for i in range(1, TK // DH):
                    ps = ps + p[:, i * DH:(i + 1) * DH]
                l = l * alpha + ps

                g = acquire(u + 1, 1)
                v = pool[slot_ref[u + 1]]
                acc = acc * alpha + jnp.dot(p.astype(jnp.bfloat16), v,
                                            preferred_element_type=jnp.float32)
                release(g)
                return m_new, l, acc

            m0 = jnp.full((8, 1), -jnp.inf, jnp.float32)
            l0 = jnp.zeros((8, DH), jnp.float32)
            a0 = jnp.zeros((8, DH), jnp.float32)
            m, l, acc = lax.fori_loop(0, nch, chunk_body, (m0, l0, a0))
            o = acc / jnp.sum(l, axis=-1, keepdims=True)
            lhs = jnp.concatenate(
                [jnp.where(row == r, o, 0.0) for r in range(rep)], axis=1
            ).astype(jnp.bfloat16)
            if layer == 0:
                @pl.when(h == 0)
                def _():
                    w_copies[2].wait()
            woh = wo_v[pl.ds(col, rep * DH), :]
            return att + jnp.dot(lhs, woh, preferred_element_type=jnp.float32)

        att = lax.fori_loop(0, hkv, head_body, jnp.zeros((8, d_model), jnp.float32))
        att = jnp.sum(att, axis=0, keepdims=True)
        return jnp.broadcast_to(att, (8, d_model))

    def mlp(x):
        xn = _layernorm_bf16(x)
        h = jnp.dot(xn, w1_v[...], preferred_element_type=jnp.float32)
        h = _rb(_rb(h) + b1_v[...].astype(jnp.float32).reshape(1, -1))
        sp = jnp.log1p(jnp.exp(-jnp.abs(h))) + jnp.where(h > 0, h, 0.0)
        act = h * jnp.tanh(sp)
        return jnp.dot(act.astype(jnp.bfloat16), w2_v[...],
                       preferred_element_type=jnp.float32)

    w_copies[0].wait()
    w_copies[1].wait()
    x = jnp.broadcast_to(x_v[...].astype(jnp.float32), (8, d_model))

    x = _rb(x + _rb(attention(0, x)))
    for c in w_copies[3:]:
        c.wait()
    x = _rb(x + _rb(mlp(x)))
    x = _rb(x + _rb(attention(1, x)))
    x = _rb(x + _rb(mlp(x)))
    o_ref[...] = x[0:1, :].astype(o_ref.dtype)


@jax.jit
def pallas_interleave_layers__gqa_block_cached__dense_activation_mish__decode_kernel(
    A_x: jax.Array,
    A_k_cache: jax.Array,
    A_v_cache: jax.Array,
    A_wq: jax.Array,
    A_wo: jax.Array,
    B_x: jax.Array,
    B_w1: jax.Array,
    B_b1: jax.Array,
    B_w2: jax.Array,
):
    B, Sq, D = A_x.shape
    _, hkv, sk, dh = A_k_cache.shape
    assert B == 1 and Sq == 1 and dh == DH and sk % TK == 0
    F = B_w1.shape[1]
    nch = sk // TK
    nu = 2 * hkv * nch
    ng = 2 * nu - NCU

    x2 = A_x.reshape(1, D)
    k2 = A_k_cache.reshape(hkv * sk, DH)
    v2 = A_v_cache.reshape(hkv * sk, DH)

    hbm = pl.BlockSpec(memory_space=pl.ANY)
    kernel = functools.partial(_kernel, hkv=hkv, nch=nch, d_model=D)
    out = pl.pallas_call(
        kernel,
        out_shape=jax.ShapeDtypeStruct((1, D), A_x.dtype),
        in_specs=[hbm] * 8,
        out_specs=pl.BlockSpec(memory_space=pltpu.VMEM),
        scratch_shapes=[
            pltpu.VMEM((NCU + NRU, TK, DH), jnp.bfloat16),
            pltpu.VMEM((1, D), jnp.bfloat16),
            pltpu.VMEM(A_wq.shape, jnp.bfloat16),
            pltpu.VMEM(A_wo.shape, jnp.bfloat16),
            pltpu.VMEM(B_w1.shape, jnp.bfloat16),
            pltpu.VMEM((F,), jnp.bfloat16),
            pltpu.VMEM(B_w2.shape, jnp.bfloat16),
            pltpu.SMEM((nu,), jnp.int32),
            pltpu.SMEM((nu,), jnp.int32),
            pltpu.SMEM((nu,), jnp.int32),
            pltpu.SMEM((ng,), jnp.int32),
            pltpu.SMEM((ng,), jnp.int32),
            pltpu.SemaphoreType.DMA((NRU,)),
            pltpu.SemaphoreType.DMA((6,)),
        ],
        compiler_params=pltpu.CompilerParams(vmem_limit_bytes=VMEM_LIMIT),
    )(x2, k2, v2, A_wq, A_wo, B_w1, B_b1, B_w2)
    return out.reshape(B, Sq, D)
```

```python
import functools

import numpy as np
import jax
import jax.numpy as jnp
from jax import lax
import jax.experimental.pallas as pl
import jax.experimental.pallas.tpu as pltpu

HQ = 32
DH = 128
EPS = 1e-5

TK = 2048
NRU = 3
NCU = 229
VMEM_LIMIT = 128 * 1024 * 1024


def _stream_count(u, nu, ns):
    return (u * (ns - 1) + (nu - 2)) // (nu - 1)


def _make_tables(nu, nc, nr):
    ns = nu - nc
    spos = [(s * (nu - 1)) // (ns - 1) for s in range(ns)]
    assert len(set(spos)) == ns
    streamed = np.zeros(nu, bool)
    streamed[spos] = True
    for u in range(nu + 1):
        assert _stream_count(u, nu, ns) == int(streamed[:u].sum())
    ng = nu + ns
    dma_unit = np.zeros(ng, np.int32)
    dma_slot = np.zeros(ng, np.int32)
    ci = 0
    si = 0
    for u in range(nu):
        if streamed[u]:
            slot = nc + si % nr
            si += 1
        else:
            slot = ci
            ci += 1
        dma_unit[u] = u
        dma_slot[u] = slot
    for j, u in enumerate(spos):
        dma_unit[nu + j] = u
        dma_slot[nu + j] = nc + (ns + j) % nr
    c0, r, r1, r2 = 0, 0, 0, ns % nr
    for u in range(nu):
        is_s = r < ns - 1
        assert is_s == bool(streamed[u])
        assert dma_slot[u] == (nc + r1 if is_s else u - c0)
        if is_s:
            assert dma_unit[nu + c0] == u and dma_slot[nu + c0] == nc + r2
        inc = int(is_s)
        r = r - (ns - 1) + (nu - 1 if is_s else 0)
        c0, r1, r2 = c0 + inc, (r1 + inc) % nr, (r2 + inc) % nr
    return dma_unit, dma_slot


def _layernorm_bf16(x):
    m = jnp.mean(x, axis=-1, keepdims=True)
    d = x - m
    v = jnp.mean(d * d, axis=-1, keepdims=True)
    return (d / jnp.sqrt(v + EPS)).astype(jnp.bfloat16)


def _rb(x):
    return x.astype(jnp.bfloat16).astype(jnp.float32)


def _kernel(x_hbm, k_hbm, v_hbm, wq_hbm, wo_hbm, w1_hbm, b1_hbm, w2_hbm,
            o_ref,
            pool, x_v, wq_v, wo_v, w1_v, b1_v, w2_v,
            slot1_ref, slot2_ref, g2_ref, dunit_ref, dslot_ref,
            sem, semw,
            *, hkv, nch, d_model):
    rep = HQ // hkv
    nu = 2 * hkv * nch
    ns = nu - NCU
    ng = nu + ns
    scale = DH ** -0.5
    tabs = _make_tables(nu, NCU, NRU)
    srcs = (k_hbm, v_hbm)

    def unit_copy(g, which):
        if isinstance(g, int):
            blk = int(tabs[0][g]) // 2
            slot = int(tabs[1][g])
            si = g % NRU
            off = blk * TK
        else:
            blk = lax.shift_right_logical(dunit_ref[g], 1)
            slot = dslot_ref[g]
            si = lax.rem(g, NRU)
            off = pl.multiple_of(blk * TK, TK)
        return pltpu.make_async_copy(srcs[which].at[pl.ds(off, TK)], pool.at[slot],
                                     sem.at[si])

    def issue(g):
        if isinstance(g, int):
            unit_copy(g, int(tabs[0][g]) % 2).start()
            return
        par = jnp.bitwise_and(dunit_ref[g], 1)

        @pl.when(par == 0)
        def _():
            unit_copy(g, 0).start()

        @pl.when(par == 1)
        def _():
            unit_copy(g, 1).start()

    w_copies = [
        pltpu.make_async_copy(x_hbm, x_v, semw.at[0]),
        pltpu.make_async_copy(wq_hbm, wq_v, semw.at[1]),
        pltpu.make_async_copy(wo_hbm, wo_v, semw.at[2]),
        pltpu.make_async_copy(w1_hbm, w1_v, semw.at[3]),
        pltpu.make_async_copy(b1_hbm, b1_v, semw.at[4]),
        pltpu.make_async_copy(w2_hbm, w2_v, semw.at[5]),
    ]
    w_copies[0].start()
    w_copies[1].start()
    for g in range(NRU):
        issue(g)
    for c in w_copies[2:]:
        c.start()

    def fill(u, carry):
        c0, r, r1, r2 = carry
        is_s = r < (ns - 1)
        s1 = jnp.where(is_s, NCU + r1, u - c0)
        s2 = jnp.where(is_s, NCU + r2, u - c0)
        slot1_ref[u] = s1
        slot2_ref[u] = s2
        g2_ref[u] = jnp.where(is_s, nu + c0, -1)
        dunit_ref[u] = u
        dslot_ref[u] = s1

        @pl.when(is_s)
        def _():
            dunit_ref[nu + c0] = u
            dslot_ref[nu + c0] = s2

        inc = is_s.astype(jnp.int32)
        r_n = r - (ns - 1) + jnp.where(is_s, nu - 1, 0)
        r1_n = jnp.where(r1 + inc == NRU, 0, r1 + inc)
        r2_n = jnp.where(r2 + inc == NRU, 0, r2 + inc)
        return c0 + inc, r_n, r1_n, r2_n

    lax.fori_loop(0, nu, fill,
                  (jnp.int32(0), jnp.int32(0), jnp.int32(0), jnp.int32(ns % NRU)))

    row = lax.broadcasted_iota(jnp.int32, (8, DH), 0)

    def attention(layer, x):
        slot_ref = slot1_ref if layer == 0 else slot2_ref
        xn = _layernorm_bf16(x)

        def acquire(u, which):
            if layer == 0:
                unit_copy(u, which).wait()
                return u
            g = g2_ref[u]

            @pl.when(g >= 0)
            def _():
                unit_copy(g, which).wait()
            return g

        def release(g):
            if layer == 0:
                issue(g + NRU)
            else:
                @pl.when(jnp.logical_and(g >= 0, g + NRU < ng))
                def _():
                    issue(g + NRU)

        def head_body(h, att):
            col = pl.multiple_of(h * (rep * DH), rep * DH)
            qf = jnp.dot(xn, wq_v[:, pl.ds(col, rep * DH)],
                         preferred_element_type=jnp.float32)
            q = jnp.zeros((8, DH), jnp.float32)
            for r in range(rep):
                q = jnp.where(row == r, qf[:, r * DH:(r + 1) * DH], q)
            q = q.astype(jnp.bfloat16)

            def chunk_body(c, carry):
                m, l, acc = carry
                u = 2 * (h * nch + c)
                g = acquire(u, 0)
                k = pool[slot_ref[u]]
                s = lax.dot_general(q, k, (((1,), (1,)), ((), ())),
                                    preferred_element_type=jnp.float32)
                release(g)
                s = s * scale
                m_new = jnp.maximum(m, jnp.max(s, axis=-1, keepdims=True))
                alpha = jnp.exp(m - m_new)
                p = jnp.exp(s - m_new)
                ps = p[:, 0:DH]
                for i in range(1, TK // DH):
                    ps = ps + p[:, i * DH:(i + 1) * DH]
                l = l * alpha + ps

                g = acquire(u + 1, 1)
                v = pool[slot_ref[u + 1]]
                acc = acc * alpha + jnp.dot(p.astype(jnp.bfloat16), v,
                                            preferred_element_type=jnp.float32)
                release(g)
                return m_new, l, acc

            m0 = jnp.full((8, 1), -jnp.inf, jnp.float32)
            l0 = jnp.zeros((8, DH), jnp.float32)
            a0 = jnp.zeros((8, DH), jnp.float32)
            m, l, acc = lax.fori_loop(0, nch, chunk_body, (m0, l0, a0))
            o = acc / jnp.sum(l, axis=-1, keepdims=True)
            lhs = jnp.concatenate(
                [jnp.where(row == r, o, 0.0) for r in range(rep)], axis=1
            ).astype(jnp.bfloat16)
            if layer == 0:
                @pl.when(h == 0)
                def _():
                    w_copies[2].wait()
            woh = wo_v[pl.ds(col, rep * DH), :]
            return att + jnp.dot(lhs, woh, preferred_element_type=jnp.float32)

        att = lax.fori_loop(0, hkv, head_body, jnp.zeros((8, d_model), jnp.float32))
        att = jnp.sum(att, axis=0, keepdims=True)
        return jnp.broadcast_to(att, (8, d_model))

    def mlp(x):
        xn = _layernorm_bf16(x)
        h = jnp.dot(xn, w1_v[...], preferred_element_type=jnp.float32)
        h = _rb(_rb(h) + b1_v[...].astype(jnp.float32).reshape(1, -1))
        sp = jnp.log1p(jnp.exp(-jnp.abs(h))) + jnp.where(h > 0, h, 0.0)
        act = h * jnp.tanh(sp)
        return jnp.dot(act.astype(jnp.bfloat16), w2_v[...],
                       preferred_element_type=jnp.float32)

    w_copies[0].wait()
    w_copies[1].wait()
    x = jnp.broadcast_to(x_v[...].astype(jnp.float32), (8, d_model))

    x = _rb(x + _rb(attention(0, x)))
    for c in w_copies[3:]:
        c.wait()
    x = _rb(x + _rb(mlp(x)))
    x = _rb(x + _rb(attention(1, x)))
    x = _rb(x + _rb(mlp(x)))
    o_ref[...] = x[0:1, :].astype(o_ref.dtype)


@jax.jit
def pallas_interleave_layers__gqa_block_cached__dense_activation_mish__decode_kernel(
    A_x: jax.Array,
    A_k_cache: jax.Array,
    A_v_cache: jax.Array,
    A_wq: jax.Array,
    A_wo: jax.Array,
    B_x: jax.Array,
    B_w1: jax.Array,
    B_b1: jax.Array,
    B_w2: jax.Array,
):
    B, Sq, D = A_x.shape
    _, hkv, sk, dh = A_k_cache.shape
    assert B == 1 and Sq == 1 and dh == DH and sk % TK == 0
    F = B_w1.shape[1]
    nch = sk // TK
    nu = 2 * hkv * nch
    ng = 2 * nu - NCU

    x2 = A_x.reshape(1, D)
    k2 = A_k_cache.reshape(hkv * sk, DH)
    v2 = A_v_cache.reshape(hkv * sk, DH)

    hbm = pl.BlockSpec(memory_space=pl.ANY)
    kernel = functools.partial(_kernel, hkv=hkv, nch=nch, d_model=D)
    out = pl.pallas_call(
        kernel,
        out_shape=jax.ShapeDtypeStruct((1, D), A_x.dtype),
        in_specs=[hbm] * 8,
        out_specs=pl.BlockSpec(memory_space=pltpu.VMEM),
        scratch_shapes=[
            pltpu.VMEM((NCU + NRU, TK, DH), jnp.bfloat16),
            pltpu.VMEM((1, D), jnp.bfloat16),
            pltpu.VMEM(A_wq.shape, jnp.bfloat16),
            pltpu.VMEM(A_wo.shape, jnp.bfloat16),
            pltpu.VMEM(B_w1.shape, jnp.bfloat16),
            pltpu.VMEM((F,), jnp.bfloat16),
            pltpu.VMEM(B_w2.shape, jnp.bfloat16),
            pltpu.SMEM((nu,), jnp.int32),
            pltpu.SMEM((nu,), jnp.int32),
            pltpu.SMEM((nu,), jnp.int32),
            pltpu.SMEM((ng,), jnp.int32),
            pltpu.SMEM((ng,), jnp.int32),
            pltpu.SemaphoreType.DMA((NRU,)),
            pltpu.SemaphoreType.DMA((6,)),
        ],
        compiler_params=pltpu.CompilerParams(vmem_limit_bytes=VMEM_LIMIT),
    )(x2, k2, v2, A_wq, A_wo, B_w1, B_b1, B_w2)
    return out.reshape(B, Sq, D)
```
